```python
import jax
import jax.numpy as jnp

def _softmax(x, axis=-1):
    return jax.nn.softmax(x, axis=axis)
def _gelu(x):
    return jax.nn.gelu(x, approximate=True)
def _silu(x):
    return jax.nn.silu(x)
def _sigmoid(x):
    return jax.nn.sigmoid(x)
def _layernorm(x, axis=-1, eps=1e-5):
    m = jnp.mean(x, axis=axis, keepdims=True)
    v = jnp.var(x, axis=axis, keepdims=True)
    return (x - m) / jnp.sqrt(v + eps)
def _scatter_add(tgt, idx, src, axis=0):
    return tgt.at[idx].add(src)
def _segment_sum(src, seg, n):
    return jax.ops.segment_sum(src, seg, n)
class _Rng:
    def __init__(self, key):
        self._k = key
    def _next(self):
        self._k, sub = jax.random.split(self._k)
        return sub
    def normal(self, shape):
        return jax.random.normal(self._next(), shape, dtype=jnp.bfloat16)
    def randint(self, lo, hi, shape):
        return jax.random.randint(self._next(), shape, lo, hi, dtype=jnp.int32)
    def uniform(self, shape, lo=0.0, hi=1.0):
        return jax.random.uniform(self._next(), shape, jnp.bfloat16, lo, hi)
    def permutation(self, n):
        return jax.random.permutation(self._next(), n)


kernel_name = 'sequential_preLN__compressed_kv_cla__moe_arch_mod__prompt'

def setup_inputs():
    _rng = _Rng(jax.random.key(int.from_bytes(__import__("os").urandom(4), "little")))
    _w = (lambda a: (lambda t: t.astype(jnp.bfloat16) if jnp.issubdtype(t.dtype, jnp.floating) else t)(jnp.asarray(a)))
    def _A_setup():
        B, H, Sq, Sk, D, M = 1, 32, 2048, 2048, 128, 1024
        Dc = 4 * D
        return {
            "x": _w((lambda *s: _rng.normal(s) * 0.05)(B, Sq, M)),
            "c_kv": _w((lambda *s: _rng.normal(s) * 0.05)(B, Sk, Dc)),
            "w_q": _w((lambda *s: _rng.normal(s) * 0.05)(M, H, D) * (M ** -0.5)),
            "w_uk": _w((lambda *s: _rng.normal(s) * 0.05)(Dc, H, D) * (Dc ** -0.5)),
            "w_uv": _w((lambda *s: _rng.normal(s) * 0.05)(Dc, H, D) * (Dc ** -0.5)),
            "w_o": _w((lambda *s: _rng.normal(s) * 0.05)(H, D, M) * ((H * D) ** -0.5)),
        }
    _A_in = _A_setup()

    def _B_setup():
        B, S, D, F, C = 1, 2048, 1024, 3584, 2
        return {
            "x": _w((lambda *s: _rng.normal(s) * 0.05)(B, S, D)),
            "w_r": _w((lambda *s: _rng.normal(s) * 0.05)(D)),
            "w_gate": _w((lambda *s: _rng.normal(s) * 0.05)(D, F)),
            "w_up": _w((lambda *s: _rng.normal(s) * 0.05)(D, F)),
            "w_down": _w((lambda *s: _rng.normal(s) * 0.05)(F, D)),
        }
    _B_in = _B_setup()

    return {
        "A_x": _A_in["x"],
        "A_c_kv": _A_in["c_kv"],
        "A_w_q": _A_in["w_q"],
        "A_w_uk": _A_in["w_uk"],
        "A_w_uv": _A_in["w_uv"],
        "A_w_o": _A_in["w_o"],
        "B_x": _B_in["x"],
        "B_w_r": _B_in["w_r"],
        "B_w_gate": _B_in["w_gate"],
        "B_w_up": _B_in["w_up"],
        "B_w_down": _B_in["w_down"],
    }

def reference(A_x, A_c_kv, A_w_q, A_w_uk, A_w_uv, A_w_o, B_x, B_w_r, B_w_gate, B_w_up, B_w_down):
    def _A_ref(x, c_kv, w_q, w_uk, w_uv, w_o):
        B, Sq, M = x.shape[0], x.shape[1], x.shape[2]
        Sk = c_kv.shape[1]
        H, D = w_q.shape[1], w_q.shape[2]
        q = jnp.einsum("bqm,mhd->bhqd", x, w_q)
        k = jnp.einsum("bkc,chd->bhkd", c_kv, w_uk)
        v = jnp.einsum("bkc,chd->bhkd", c_kv, w_uv)
        scores = jnp.einsum("bhqd,bhkd->bhqk", q, k) * (D ** -0.5)
        off = Sk - Sq
        qi = jnp.arange(Sq)[:, None]
        kj = jnp.arange(Sk)[None, :]
        cmask = kj <= (qi + off)
        scores = jnp.where(cmask[None, None], scores, -1e9)
        p = _softmax(scores, axis=-1)
        ctx = jnp.einsum("bhqk,bhkd->bhqd", p, v)
        return jnp.einsum("bhqd,hdm->bqm", ctx, w_o)

    def _B_ref(x, w_r, w_gate, w_up, w_down):
        B, S, D = x.shape
        C = 2
        r = x @ w_r
        idx = jnp.argsort(-r, axis=-1)[:, :C]
        idx_e = jnp.repeat(idx.reshape(B, C, 1), D, axis=2)
        x_sel = jnp.take_along_axis(x, idx_e, axis=1)
        g = _silu(x_sel @ w_gate)
        u = x_sel @ w_up
        y = (g * u) @ w_down
        r_sel = _sigmoid(jnp.take_along_axis(r, idx, axis=1))
        y = y * r_sel.reshape(B, C, 1)
        b_off = (jnp.arange(B) * S).reshape(B, 1)
        flat_idx = (idx + b_off).reshape(B * C)
        zero = (x * 0.0).reshape(B * S, D)
        upd = _scatter_add(zero, flat_idx, y.reshape(B * C, D), axis=0)
        return x + upd.reshape(B, S, D)

    x = A_x
    h = x + _A_ref(_layernorm(x, axis=-1), A_c_kv, A_w_q, A_w_uk, A_w_uv, A_w_o)
    h2 = h + _B_ref(_layernorm(h, axis=-1), B_w_r, B_w_gate, B_w_up, B_w_down)
    return h2
```

```python
import functools
import numpy as np
import jax
import jax.numpy as jnp
from jax import lax
import jax.experimental.pallas as pl
import jax.experimental.pallas.tpu as pltpu

S, M, H, D, DC, F = 2048, 1024, 32, 128, 512, 3584
BQ = 256
NQ = S // BQ
LOG2E = float(np.log2(np.e))
NT = (((1,), (1,)), ((), ()))
f32, bf16 = jnp.float32, jnp.bfloat16


def _ln(v):
    m = jnp.mean(v, axis=-1, keepdims=True)
    d = v - m
    var = jnp.mean(d * d, axis=-1, keepdims=True)
    return d * lax.rsqrt(var + 1e-5)


def _kernel(x_ref, c_ref, wq_ref, wk_ref, wv_ref, wr_ref, wo_hbm, wg_hbm, wu_hbm, wd_hbm,
            o_hbm, xn_ref, ctx_ref, wo_ref, wg_ref, wu_ref, wd_ref, h_ref, st_ref, r_ref, wsem, osem):
    hd = pl.program_id(0)

    def wcopies():
        return [pltpu.make_async_copy(s, d, wsem.at[i]) for i, (s, d) in
                enumerate([(wo_hbm, wo_ref), (wg_hbm, wg_ref), (wu_hbm, wu_ref), (wd_hbm, wd_ref)])]

    @pl.when(hd == 0)
    def _():
        for cp in wcopies():
            cp.start()

        def body(i, carry):
            rows = pl.ds(pl.multiple_of(i * BQ, BQ), BQ)
            xn_ref[rows, :] = _ln(x_ref[rows, :].astype(f32)).astype(bf16)
            return carry
        lax.fori_loop(0, NQ, body, 0)

    c = c_ref[...]
    k = jnp.dot(c, wk_ref[...], preferred_element_type=f32).astype(bf16)
    v = jnp.dot(c, wv_ref[...], preferred_element_type=f32).astype(bf16)
    q = (jnp.dot(xn_ref[...], wq_ref[...], preferred_element_type=f32) * (D ** -0.5 * LOG2E)).astype(bf16)
    rr = lax.broadcasted_iota(jnp.int32, (BQ, BQ), 0)
    cc = lax.broadcasted_iota(jnp.int32, (BQ, BQ), 1)
    tri = cc <= rr
    for i in range(NQ):
        n = (i + 1) * BQ
        qi = q[i * BQ:n]
        sd = lax.dot_general(qi, k[i * BQ:n], NT, preferred_element_type=f32)
        sd = jnp.where(tri, sd, -1e9 * LOG2E)
        m = jnp.max(sd, axis=-1, keepdims=True)
        if i > 0:
            so = lax.dot_general(qi, k[:i * BQ], NT, preferred_element_type=f32)
            m = jnp.maximum(m, jnp.max(so, axis=-1, keepdims=True))
        pd = jnp.exp2(sd - m)
        l = jnp.sum(pd, axis=-1, keepdims=True)
        o = jnp.dot(pd.astype(bf16), v[i * BQ:n], preferred_element_type=f32)
        if i > 0:
            po = jnp.exp2(so - m)
            l = l + jnp.sum(po, axis=-1, keepdims=True)
            o = o + jnp.dot(po.astype(bf16), v[:i * BQ], preferred_element_type=f32)
        ctx_ref[hd, i * BQ:n, :] = (o / l).astype(bf16)

    @pl.when(hd == H - 1)
    def _():
        cps = wcopies()
        cps[0].wait()
        wr = wr_ref[...].astype(f32)

        def ocopy(i):
            rows = pl.ds(pl.multiple_of(i * BQ, BQ), BQ)
            return pltpu.make_async_copy(st_ref.at[rows, :], o_hbm.at[rows, :], osem.at[i])

        def body(i, carry):
            rows = pl.ds(pl.multiple_of(i * BQ, BQ), BQ)
            ctx = jnp.concatenate([ctx_ref[j, rows, :] for j in range(H)], axis=1)
            a = jnp.dot(ctx, wo_ref[...], preferred_element_type=f32).astype(bf16)
            h = (x_ref[rows, :].astype(f32) + a.astype(f32)).astype(bf16)
            ln = _ln(h.astype(f32)).astype(bf16)
            r = jnp.sum(ln.astype(f32) * wr, axis=-1, keepdims=True).astype(bf16).astype(f32)
            r_ref[rows, :] = r
            h_ref[rows, :] = h
            xn_ref[rows, :] = ln
            st_ref[rows, :] = (h.astype(f32) + ln.astype(f32)).astype(bf16)
            ocopy(i).start()
            return carry
        lax.fori_loop(0, NQ, body, 0)

        r = r_ref[...]
        ids = lax.broadcasted_iota(jnp.int32, (S, 1), 0)
        m1 = jnp.max(r)
        i1 = jnp.min(jnp.where(r == m1, ids, S))
        r2 = jnp.where(ids == i1, -jnp.inf, r)
        m2 = jnp.max(r2)
        i2 = jnp.min(jnp.where(r2 == m2, ids, S))
        i1 = jnp.minimum(i1, S - 1)
        i2 = jnp.minimum(i2, S - 1)
        b1 = pl.multiple_of((i1 // 16) * 16, 16)
        b2 = pl.multiple_of((i2 // 16) * 16, 16)
        rid = lax.broadcasted_iota(jnp.int32, (16, 1), 0)
        t1 = xn_ref[pl.ds(b1, 16), :].astype(f32)
        t2 = xn_ref[pl.ds(b2, 16), :].astype(f32)
        x1 = jnp.sum(jnp.where(rid == i1 - b1, t1, 0.0), axis=0, keepdims=True)
        x2 = jnp.sum(jnp.where(rid == i2 - b2, t2, 0.0), axis=0, keepdims=True)
        xs = jnp.where(rid == 0, x1, jnp.where(rid == 1, x2, 0.0)).astype(bf16)
        for cp in cps[1:]:
            cp.wait()
        g = jnp.dot(xs, wg_ref[...], preferred_element_type=f32).astype(bf16).astype(f32)
        u = jnp.dot(xs, wu_ref[...], preferred_element_type=f32).astype(bf16).astype(f32)
        g = (g * jax.nn.sigmoid(g)).astype(bf16).astype(f32)
        y = jnp.dot((g * u).astype(bf16), wd_ref[...], preferred_element_type=f32).astype(bf16).astype(f32)
        s1 = jax.nn.sigmoid(jnp.full((1, M), m1, f32)).astype(bf16).astype(f32)
        s2 = jax.nn.sigmoid(jnp.full((1, M), m2, f32)).astype(bf16).astype(f32)
        y1 = (y[0:1] * s1).astype(bf16).astype(f32)
        y2 = (y[1:2] * s2).astype(bf16).astype(f32)
        for i in range(NQ):
            ocopy(i).wait()
        for (bb, ii, tt, yy) in ((b1, i1, t1, y1), (b2, i2, t2, y2)):
            rows = pl.ds(bb, 16)
            new = (h_ref[rows, :].astype(f32) + (tt + yy).astype(bf16).astype(f32)).astype(bf16)
            st_ref[rows, :] = jnp.where(rid == ii - bb, new, st_ref[rows, :])
            cp = pltpu.make_async_copy(st_ref.at[rows, :], o_hbm.at[rows, :], osem.at[0])
            cp.start()
            cp.wait()


@jax.jit
def pallas_sequential_preLN__compressed_kv_cla__moe_arch_mod__prompt_kernel(
        A_x, A_c_kv, A_w_q, A_w_uk, A_w_uv, A_w_o, B_x, B_w_r, B_w_gate, B_w_up, B_w_down):
    x = A_x.reshape(S, M)
    c = A_c_kv.reshape(S, DC)
    wq = A_w_q.reshape(M, H * D)
    wk = A_w_uk.reshape(DC, H * D)
    wv = A_w_uv.reshape(DC, H * D)
    wo = A_w_o.reshape(H * D, M)
    wr = B_w_r.reshape(1, M)
    anyspec = pl.BlockSpec(memory_space=pl.ANY)
    out = pl.pallas_call(
        _kernel,
        grid=(H,),
        in_specs=[
            pl.BlockSpec((S, M), lambda h: (0, 0), pipeline_mode=pl.Buffered(1)),
            pl.BlockSpec((S, DC), lambda h: (0, 0), pipeline_mode=pl.Buffered(1)),
            pl.BlockSpec((M, D), lambda h: (0, h)),
            pl.BlockSpec((DC, D), lambda h: (0, h)),
            pl.BlockSpec((DC, D), lambda h: (0, h)),
            pl.BlockSpec((1, M), lambda h: (0, 0)),
            anyspec, anyspec, anyspec, anyspec,
        ],
        out_specs=anyspec,
        out_shape=jax.ShapeDtypeStruct((S, M), bf16),
        scratch_shapes=[
            pltpu.VMEM((S, M), bf16),
            pltpu.VMEM((H, S, D), bf16),
            pltpu.VMEM((H * D, M), bf16),
            pltpu.VMEM((M, F), bf16),
            pltpu.VMEM((M, F), bf16),
            pltpu.VMEM((F, M), bf16),
            pltpu.VMEM((S, M), bf16),
            pltpu.VMEM((S, M), bf16),
            pltpu.VMEM((S, 1), f32),
            pltpu.SemaphoreType.DMA((4,)),
            pltpu.SemaphoreType.DMA((NQ,)),
        ],
        compiler_params=pltpu.CompilerParams(
            dimension_semantics=("arbitrary",), vmem_limit_bytes=120 * 1024 * 1024),
    )(x, c, wq, wk, wv, wr, wo, B_w_gate, B_w_up, B_w_down)
    return out.reshape(1, S, M)
```

```python
import os
import numpy as np
import jax
import jax.numpy as jnp
from jax import lax
import jax.experimental.pallas as pl
import jax.experimental.pallas.tpu as pltpu

S, M, H, D, DC, F = 2048, 1024, 32, 128, 512, 3584
MODE = os.environ.get("MODE", "h")
BQ = int("256")
PB = int("256")
RB = 256
LOG2E = float(np.log2(np.e))
NT = (((1,), (1,)), ((), ()))
f32, bf16, u32 = jnp.float32, jnp.bfloat16, jnp.uint32
HG = 16


def _ln(v):
    m = jnp.mean(v, axis=-1, keepdims=True)
    d = v - m
    var = jnp.mean(d * d, axis=-1, keepdims=True)
    return d * lax.rsqrt(var + 1e-5)


def _dot(a, b):
    return jnp.dot(a, b, preferred_element_type=f32)


def _dot_nt(a, b):
    return lax.dot_general(a, b, NT, preferred_element_type=f32)


def _kernel(x_hbm, c_hbm, wq_hbm, wk_hbm, wv_hbm, wr_ref, wo_hbm, wg_hbm, wu_hbm, wd_hbm,
            o_hbm,
            x_ref, c_ref, nq_ref, nk_ref, nv_ref, uq_ref, uk_ref, uv_ref, qkv_ref,
            xn_ref, ctx_ref, wo_ref, wg_ref, wu_ref, wd_ref, h_ref, st_ref, r_ref,
            isem, nsem, wsem, osem):
    step = pl.program_id(0)

    def nat_copy(i, g):
        src, dst = ((wq_hbm, nq_ref), (wk_hbm, nk_ref), (wv_hbm, nv_ref))[i]
        return pltpu.make_async_copy(src.at[:, pl.ds(g * HG, HG), :], dst, nsem.at[i])

    def in_copy(i):
        src, dst = ((x_hbm, x_ref), (c_hbm, c_ref))[i]
        return pltpu.make_async_copy(src, dst, isem.at[i])

    def w_copy(i):
        src, dst = ((wo_hbm, wo_ref), (wg_hbm, wg_ref), (wu_hbm, wu_ref), (wd_hbm, wd_ref))[i]
        return pltpu.make_async_copy(src, dst, wsem.at[i])

    def stage(nat, dst):
        def body(i, carry):
            r = pl.multiple_of(i * 128, 128)
            v = pltpu.bitcast(nat[pl.ds(r, 128)], u32)
            dst[pl.ds(pl.multiple_of(i * 1024, 1024), 1024), :] = v.reshape(1024, 128)
            return carry
        lax.fori_loop(0, nat.shape[0] // 128, body, 0)

    def head_w(ref, hd):
        hl = hd % HG
        u = ref[pl.ds(hl // 2, ref.shape[0] // 8, stride=8), :]
        sh = jnp.asarray(16 * (1 - hl % 2)).astype(u32)
        return pltpu.bitcast((u << sh) & u32(0xFFFF0000), f32).astype(bf16)

    def proj(hd):
        slot = hd % 2
        wq, wk, wv = head_w(uq_ref, hd), head_w(uk_ref, hd), head_w(uv_ref, hd)

        def chunk(i):
            rows = slice(i * PB, (i + 1) * PB)
            c = c_ref[rows, :]
            qkv_ref[slot, 1, rows, :] = _dot(c, wk).astype(bf16)
            qkv_ref[slot, 2, rows, :] = _dot(c, wv).astype(bf16)
            qkv_ref[slot, 0, rows, :] = (_dot(xn_ref[rows, :], wq) * (D ** -0.5 * LOG2E)).astype(bf16)
        return chunk

    def attn_block(hd, r0, r1, c1):
        slot = hd % 2
        n = r1 - r0
        q = qkv_ref[slot, 0, r0:r1, :]
        parts = []
        c0 = c1 - n
        if c0 > 0:
            parts.append(_dot_nt(q, qkv_ref[slot, 1, 0:c0, :]))
        rr = lax.broadcasted_iota(jnp.int32, (n, n), 0)
        cc = lax.broadcasted_iota(jnp.int32, (n, n), 1)
        sd = _dot_nt(q, qkv_ref[slot, 1, c0:c1, :])
        parts.append(jnp.where(cc <= rr, sd, -1e9 * LOG2E))
        s = jnp.concatenate(parts, axis=1) if len(parts) > 1 else parts[0]
        m = jnp.max(s, axis=-1, keepdims=True)
        p = jnp.exp2(s - m)
        l = jnp.sum(p, axis=-1, keepdims=True)
        o = _dot(p.astype(bf16), qkv_ref[slot, 2, 0:c1, :])
        ctx_ref[hd, r0:r1, :] = (o / l).astype(bf16)

    def attn_and_proj(hd, with_proj):
        chunk = proj(hd + 1) if with_proj else None
        nb = S // BQ
        npb = S // PB
        done = 0
        for i in range(nb):
            if with_proj:
                while done < npb and done * nb <= i * npb:
                    chunk(done)
                    done += 1
            attn_block(hd, i * BQ, (i + 1) * BQ, (i + 1) * BQ)
        if with_proj:
            while done < npb:
                chunk(done)
                done += 1

    @pl.when(step == 0)
    def _():
        in_copy(1).start()
        nat_copy(1, 0).start()
        nat_copy(2, 0).start()
        in_copy(0).start()
        nat_copy(0, 0).start()
        w_copy(0).start()
        in_copy(1).wait()
        nat_copy(1, 0).wait()
        stage(nk_ref, uk_ref)
        nat_copy(1, 1).start()
        nat_copy(2, 0).wait()
        stage(nv_ref, uv_ref)
        nat_copy(2, 1).start()
        in_copy(0).wait()

        def body(i, carry):
            rows = pl.ds(pl.multiple_of(i * RB, RB), RB)
            xn_ref[rows, :] = _ln(x_ref[rows, :].astype(f32)).astype(bf16)
            return carry
        lax.fori_loop(0, S // RB, body, 0)
        nat_copy(0, 0).wait()
        stage(nq_ref, uq_ref)
        nat_copy(0, 1).start()
        for i in range(1, 4):
            w_copy(i).start()
        chunk = proj(0)
        for i in range(S // PB):
            chunk(i)

    @pl.when(step == HG - 1)
    def _():
        for i in range(3):
            nat_copy(i, 1).wait()
        stage(nk_ref, uk_ref)
        stage(nv_ref, uv_ref)
        stage(nq_ref, uq_ref)

    @pl.when(step < H - 1)
    def _():
        attn_and_proj(step, True)

    @pl.when(step == H - 1)
    def _():
        attn_and_proj(step, False)
        w_copy(0).wait()
        wr = wr_ref[...].astype(f32)
        NQ = S // RB

        def ocopy(i):
            rows = pl.ds(pl.multiple_of(i * RB, RB), RB)
            return pltpu.make_async_copy(st_ref.at[rows, :], o_hbm.at[rows, :], osem.at[i])

        def body(i, carry):
            rows = pl.ds(pl.multiple_of(i * RB, RB), RB)
            ctx = jnp.concatenate([ctx_ref[j, rows, :] for j in range(H)], axis=1)
            a = _dot(ctx, wo_ref[...]).astype(bf16)
            h = (x_ref[rows, :].astype(f32) + a.astype(f32)).astype(bf16)
            ln = _ln(h.astype(f32)).astype(bf16)
            r = jnp.sum(ln.astype(f32) * wr, axis=-1, keepdims=True).astype(bf16).astype(f32)
            r_ref[rows, :] = r
            h_ref[rows, :] = h
            xn_ref[rows, :] = ln
            st_ref[rows, :] = (h.astype(f32) + ln.astype(f32)).astype(bf16)
            ocopy(i).start()
            return carry
        lax.fori_loop(0, NQ, body, 0)

        r = r_ref[...]
        ids = lax.broadcasted_iota(jnp.int32, (S, 1), 0)
        m1 = jnp.max(r)
        i1 = jnp.min(jnp.where(r == m1, ids, S))
        r2 = jnp.where(ids == i1, -jnp.inf, r)
        m2 = jnp.max(r2)
        i2 = jnp.min(jnp.where(r2 == m2, ids, S))
        i1 = jnp.minimum(i1, S - 1)
        i2 = jnp.minimum(i2, S - 1)
        b1 = pl.multiple_of((i1 // 16) * 16, 16)
        b2 = pl.multiple_of((i2 // 16) * 16, 16)
        rid = lax.broadcasted_iota(jnp.int32, (16, 1), 0)
        t1 = xn_ref[pl.ds(b1, 16), :].astype(f32)
        t2 = xn_ref[pl.ds(b2, 16), :].astype(f32)
        x1 = jnp.sum(jnp.where(rid == i1 - b1, t1, 0.0), axis=0, keepdims=True)
        x2 = jnp.sum(jnp.where(rid == i2 - b2, t2, 0.0), axis=0, keepdims=True)
        xs = jnp.where(rid == 0, x1, jnp.where(rid == 1, x2, 0.0)).astype(bf16)
        for i in range(1, 4):
            w_copy(i).wait()
        g = _dot(xs, wg_ref[...]).astype(bf16).astype(f32)
        u = _dot(xs, wu_ref[...]).astype(bf16).astype(f32)
        g = (g * jax.nn.sigmoid(g)).astype(bf16).astype(f32)
        y = _dot((g * u).astype(bf16), wd_ref[...]).astype(bf16).astype(f32)
        s1 = jax.nn.sigmoid(jnp.full((1, M), m1, f32)).astype(bf16).astype(f32)
        s2 = jax.nn.sigmoid(jnp.full((1, M), m2, f32)).astype(bf16).astype(f32)
        y1 = (y[0:1] * s1).astype(bf16).astype(f32)
        y2 = (y[1:2] * s2).astype(bf16).astype(f32)
        for i in range(NQ):
            ocopy(i).wait()
        for (bb, ii, tt, yy) in ((b1, i1, t1, y1), (b2, i2, t2, y2)):
            rows = pl.ds(bb, 16)
            new = (h_ref[rows, :].astype(f32) + (tt + yy).astype(bf16).astype(f32)).astype(bf16)
            st_ref[rows, :] = jnp.where(rid == ii - bb, new, st_ref[rows, :])
            cp = pltpu.make_async_copy(st_ref.at[rows, :], o_hbm.at[rows, :], osem.at[0])
            cp.start()
            cp.wait()


@jax.jit
def pallas_sequential_preLN__compressed_kv_cla__moe_arch_mod__prompt_kernel(
        A_x, A_c_kv, A_w_q, A_w_uk, A_w_uv, A_w_o, B_x, B_w_r, B_w_gate, B_w_up, B_w_down):
    x = A_x.reshape(S, M)
    c = A_c_kv.reshape(S, DC)
    wo = A_w_o.reshape(H * D, M)
    wr = B_w_r.reshape(1, M)
    anyspec = pl.BlockSpec(memory_space=pl.ANY)
    out = pl.pallas_call(
        _kernel,
        grid=(H,),
        in_specs=[anyspec] * 5 + [pl.BlockSpec((1, M), lambda h: (0, 0))] + [anyspec] * 4,
        out_specs=anyspec,
        out_shape=jax.ShapeDtypeStruct((S, M), bf16),
        scratch_shapes=[
            pltpu.VMEM((S, M), bf16),
            pltpu.VMEM((S, DC), bf16),
            pltpu.VMEM((M, HG, D), bf16),
            pltpu.VMEM((DC, HG, D), bf16),
            pltpu.VMEM((DC, HG, D), bf16),
            pltpu.VMEM((M * 8, D), u32),
            pltpu.VMEM((DC * 8, D), u32),
            pltpu.VMEM((DC * 8, D), u32),
            pltpu.VMEM((2, 3, S, D), bf16),
            pltpu.VMEM((S, M), bf16),
            pltpu.VMEM((H, S, D), bf16),
            pltpu.VMEM((H * D, M), bf16),
            pltpu.VMEM((M, F), bf16),
            pltpu.VMEM((M, F), bf16),
            pltpu.VMEM((F, M), bf16),
            pltpu.VMEM((S, M), bf16),
            pltpu.VMEM((S, M), bf16),
            pltpu.VMEM((S, 1), f32),
            pltpu.SemaphoreType.DMA((2,)),
            pltpu.SemaphoreType.DMA((3,)),
            pltpu.SemaphoreType.DMA((4,)),
            pltpu.SemaphoreType.DMA((S // RB,)),
        ],
        compiler_params=pltpu.CompilerParams(
            dimension_semantics=("arbitrary",), vmem_limit_bytes=126 * 1024 * 1024),
    )(x, c, A_w_q, A_w_uk, A_w_uv, wr, wo, B_w_gate, B_w_up, B_w_down)
    return out.reshape(1, S, M)
```

```python
import os
import numpy as np
import jax
import jax.numpy as jnp
from jax import lax
import jax.experimental.pallas as pl
import jax.experimental.pallas.tpu as pltpu

S, M, H, D, DC, F = 2048, 1024, 32, 128, 512, 3584
MODE = os.environ.get("MODE", "h")
BQ = int(os.environ.get("BQ", "256"))
PB = int(os.environ.get("PB", "256"))
RB = int(os.environ.get("RB", "256"))
NH = int(os.environ.get("NH", "32"))
ORDER = os.environ.get("ORDER", "q7,e0,p,q6,p,e7,p,q5,e6,p,q4,e5,p,q3,e4,p,q2,e3,p,q1,e2,p,N,e1")
CB = int(os.environ.get("CB", "0"))
NOP = int(os.environ.get("NOP", str(2048 // RB)))
NOFFN = int(os.environ.get("NOFFN", "0"))
LOG2E = float(np.log2(np.e))
NT = (((1,), (1,)), ((), ()))
f32, bf16, u32 = jnp.float32, jnp.bfloat16, jnp.uint32
HG = 16


def _ln(v):
    m = jnp.mean(v, axis=-1, keepdims=True)
    d = v - m
    var = jnp.mean(d * d, axis=-1, keepdims=True)
    return d * lax.rsqrt(var + 1e-5)


def _dot(a, b):
    return jnp.dot(a, b, preferred_element_type=f32)


def _dot_nt(a, b):
    return lax.dot_general(a, b, NT, preferred_element_type=f32)


def _kernel(x_hbm, c_hbm, wq_hbm, wk_hbm, wv_hbm, wr_ref, wo_hbm, wg_hbm, wu_hbm, wd_hbm,
            o_hbm,
            x_ref, c_ref, nq_ref, nk_ref, nv_ref, uq_ref, uk_ref, uv_ref, qkv_ref, sn_ref, sb_ref, mn_ref,
            xn_ref, ctx_ref, wo_ref, wg_ref, wu_ref, wd_ref, h_ref, st_ref, r_ref,
            isem, nsem, wsem, osem):
    step = pl.program_id(0)

    def nat_copy(i, g):
        src, dst = ((wq_hbm, nq_ref), (wk_hbm, nk_ref), (wv_hbm, nv_ref))[i]
        return pltpu.make_async_copy(src.at[:, pl.ds(g * HG, HG), :], dst, nsem.at[i])

    def in_copy(i):
        src, dst = ((x_hbm, x_ref), (c_hbm, c_ref))[i]
        return pltpu.make_async_copy(src, dst, isem.at[i])

    def w_copy(i):
        src, dst = ((wo_hbm, wo_ref), (wg_hbm, wg_ref), (wu_hbm, wu_ref), (wd_hbm, wd_ref))[i]
        return pltpu.make_async_copy(src, dst, wsem.at[i])

    def stage(nat, dst):
        def body(i, carry):
            r = pl.multiple_of(i * 128, 128)
            v = pltpu.bitcast(nat[pl.ds(r, 128)], u32)
            dst[pl.ds(pl.multiple_of(i * 1024, 1024), 1024), :] = v.reshape(1024, 128)
            return carry
        lax.fori_loop(0, nat.shape[0] // 128, body, 0)

    def head_w(ref, hd):
        hl = hd % HG
        u = ref[pl.ds(hl // 2, ref.shape[0] // 8, stride=8), :]
        sh = jnp.asarray(16 * (1 - hl % 2)).astype(u32)
        return pltpu.bitcast((u << sh) & u32(0xFFFF0000), f32).astype(bf16)

    def proj(hd):
        slot = hd % 2
        wq, wk, wv = head_w(uq_ref, hd), head_w(uk_ref, hd), head_w(uv_ref, hd)

        def chunk(i):
            rows = slice(i * PB, (i + 1) * PB)
            c = c_ref[rows, :]
            qkv_ref[slot, 1, rows, :] = _dot(c, wk).astype(bf16)
            qkv_ref[slot, 2, rows, :] = _dot(c, wv).astype(bf16)
            qkv_ref[slot, 0, rows, :] = (_dot(xn_ref[rows, :], wq) * (D ** -0.5 * LOG2E)).astype(bf16)
        return chunk

    HB = BQ // 2

    def scores(hd, i):
        slot = hd % 2
        r0, r1 = i * BQ, (i + 1) * BQ
        rm = r0 + HB
        q = qkv_ref[slot, 0, r0:r1, :]
        neg = -1e9 * LOG2E
        rr = lax.broadcasted_iota(jnp.int32, (BQ, HB), 0)
        cc = lax.broadcasted_iota(jnp.int32, (BQ, HB), 1)
        parts = []
        if r0 > 0:
            parts.append(_dot_nt(q, qkv_ref[slot, 1, 0:r0, :]))
        parts.append(jnp.where(cc <= rr, _dot_nt(q, qkv_ref[slot, 1, r0:rm, :]), neg))
        sa = jnp.concatenate(parts, axis=1) if len(parts) > 1 else parts[0]
        sb = jnp.where(cc[:HB] <= rr[:HB], _dot_nt(q[HB:], qkv_ref[slot, 1, rm:r1, :]), neg)
        ma = jnp.max(sa, axis=-1, keepdims=True)
        mb = jnp.maximum(ma[HB:], jnp.max(sb, axis=-1, keepdims=True))
        return sa, sb, jnp.concatenate([ma[:HB], mb], axis=0)

    def carry_scores(hd):
        sa, sb, m = scores(hd, CB)
        sn_ref[...] = sa
        sb_ref[...] = sb
        mn_ref[...] = m

    def softmax_pv(hd, i, sa, sb, m):
        slot = hd % 2
        r0, r1 = i * BQ, (i + 1) * BQ
        rm = r0 + HB
        pa = jnp.exp2(sa - m)
        pb = jnp.exp2(sb - m[HB:])
        la = jnp.sum(pa, axis=-1, keepdims=True)
        lb = la[HB:] + jnp.sum(pb, axis=-1, keepdims=True)
        oa = _dot(pa.astype(bf16), qkv_ref[slot, 2, 0:rm, :])
        ob = oa[HB:] + _dot(pb.astype(bf16), qkv_ref[slot, 2, rm:r1, :])
        ctx_ref[hd, r0:rm, :] = (oa[:HB] / la[:HB]).astype(bf16)
        ctx_ref[hd, rm:r1, :] = (ob / lb).astype(bf16)

    def attn_and_proj(hd, with_proj):
        chunk = proj(hd + 1) if with_proj else None
        done = 0
        pend = {}
        for tok in ORDER.split(","):
            if tok == "p":
                if with_proj:
                    chunk(done)
                done += 1
            elif tok == "N":
                if with_proj:
                    carry_scores(hd + 1)
            elif tok[0] == "q":
                pend[int(tok[1])] = scores(hd, int(tok[1]))
            else:
                i = int(tok[1])
                softmax_pv(hd, i, *(pend[i] if i in pend else (sn_ref[...], sb_ref[...], mn_ref[...])))
        assert done == S // PB

    @pl.when(step == 0)
    def _():
        in_copy(1).start()
        nat_copy(1, 0).start()
        nat_copy(2, 0).start()
        in_copy(0).start()
        nat_copy(0, 0).start()
        w_copy(0).start()
        in_copy(1).wait()
        nat_copy(1, 0).wait()
        stage(nk_ref, uk_ref)
        nat_copy(1, 1).start()
        nat_copy(2, 0).wait()
        stage(nv_ref, uv_ref)
        nat_copy(2, 1).start()
        in_copy(0).wait()

        def body(i, carry):
            rows = pl.ds(pl.multiple_of(i * RB, RB), RB)
            xn_ref[rows, :] = _ln(x_ref[rows, :].astype(f32)).astype(bf16)
            return carry
        lax.fori_loop(0, S // RB, body, 0)
        nat_copy(0, 0).wait()
        stage(nq_ref, uq_ref)
        nat_copy(0, 1).start()
        for i in range(1, 4):
            w_copy(i).start()
        chunk = proj(0)
        for i in range(S // PB):
            chunk(i)
        carry_scores(0)

    @pl.when(step == HG - 1)
    def _():
        for i in range(3):
            nat_copy(i, 1).wait()
        stage(nk_ref, uk_ref)
        stage(nv_ref, uv_ref)
        stage(nq_ref, uq_ref)

    @pl.when(step < NH - 1)
    def _():
        attn_and_proj(step, True)

    @pl.when(step == NH - 1)
    def _():
        attn_and_proj(step, False)
        w_copy(0).wait()
        wr = wr_ref[...].astype(f32)
        NQ = S // RB

        def ocopy(i):
            rows = pl.ds(pl.multiple_of(i * RB, RB), RB)
            return pltpu.make_async_copy(st_ref.at[rows, :], o_hbm.at[rows, :], osem.at[i])

        def body(i, carry):
            rows = pl.ds(pl.multiple_of(i * RB, RB), RB)
            ctx = jnp.concatenate([ctx_ref[j, rows, :] for j in range(H)], axis=1)
            a = _dot(ctx, wo_ref[...]).astype(bf16)
            h = (x_ref[rows, :].astype(f32) + a.astype(f32)).astype(bf16)
            ln = _ln(h.astype(f32)).astype(bf16)
            r = jnp.sum(ln.astype(f32) * wr, axis=-1, keepdims=True).astype(bf16).astype(f32)
            r_ref[rows, :] = r
            h_ref[rows, :] = h
            xn_ref[rows, :] = ln
            st_ref[rows, :] = (h.astype(f32) + ln.astype(f32)).astype(bf16)
            ocopy(i).start()
            return carry
        lax.fori_loop(0, NOP, body, 0)

        r = r_ref[...]
        ids = lax.broadcasted_iota(jnp.int32, (S, 1), 0)
        m1 = jnp.max(r)
        i1 = jnp.min(jnp.where(r == m1, ids, S))
        r2 = jnp.where(ids == i1, -jnp.inf, r)
        m2 = jnp.max(r2)
        i2 = jnp.min(jnp.where(r2 == m2, ids, S))
        i1 = jnp.minimum(i1, S - 1)
        i2 = jnp.minimum(i2, S - 1)
        b1 = pl.multiple_of((i1 // 16) * 16, 16)
        b2 = pl.multiple_of((i2 // 16) * 16, 16)
        rid = lax.broadcasted_iota(jnp.int32, (16, 1), 0)
        t1 = xn_ref[pl.ds(b1, 16), :].astype(f32)
        t2 = xn_ref[pl.ds(b2, 16), :].astype(f32)
        x1 = jnp.sum(jnp.where(rid == i1 - b1, t1, 0.0), axis=0, keepdims=True)
        x2 = jnp.sum(jnp.where(rid == i2 - b2, t2, 0.0), axis=0, keepdims=True)
        xs = jnp.where(rid == 0, x1, jnp.where(rid == 1, x2, 0.0)).astype(bf16)
        for i in range(1, 4):
            w_copy(i).wait()
        if not NOFFN:
            g = _dot(xs, wg_ref[...]).astype(bf16).astype(f32)
            u = _dot(xs, wu_ref[...]).astype(bf16).astype(f32)
            g = (g * jax.nn.sigmoid(g)).astype(bf16).astype(f32)
            y = _dot((g * u).astype(bf16), wd_ref[...]).astype(bf16).astype(f32)
        else:
            y = xs.astype(f32)
        s1 = jax.nn.sigmoid(jnp.full((1, M), m1, f32)).astype(bf16).astype(f32)
        s2 = jax.nn.sigmoid(jnp.full((1, M), m2, f32)).astype(bf16).astype(f32)
        y1 = (y[0:1] * s1).astype(bf16).astype(f32)
        y2 = (y[1:2] * s2).astype(bf16).astype(f32)
        for i in range(NOP):
            ocopy(i).wait()
        for (bb, ii, tt, yy) in ((b1, i1, t1, y1), (b2, i2, t2, y2)):
            rows = pl.ds(bb, 16)
            new = (h_ref[rows, :].astype(f32) + (tt + yy).astype(bf16).astype(f32)).astype(bf16)
            st_ref[rows, :] = jnp.where(rid == ii - bb, new, st_ref[rows, :])
            cp = pltpu.make_async_copy(st_ref.at[rows, :], o_hbm.at[rows, :], osem.at[0])
            cp.start()
            cp.wait()


@jax.jit
def pallas_sequential_preLN__compressed_kv_cla__moe_arch_mod__prompt_kernel(
        A_x, A_c_kv, A_w_q, A_w_uk, A_w_uv, A_w_o, B_x, B_w_r, B_w_gate, B_w_up, B_w_down):
    x = A_x.reshape(S, M)
    c = A_c_kv.reshape(S, DC)
    wo = A_w_o.reshape(H * D, M)
    wr = B_w_r.reshape(1, M)
    anyspec = pl.BlockSpec(memory_space=pl.ANY)
    out = pl.pallas_call(
        _kernel,
        grid=(NH,),
        in_specs=[anyspec] * 5 + [pl.BlockSpec((1, M), lambda h: (0, 0))] + [anyspec] * 4,
        out_specs=anyspec,
        out_shape=jax.ShapeDtypeStruct((S, M), bf16),
        scratch_shapes=[
            pltpu.VMEM((S, M), bf16),
            pltpu.VMEM((S, DC), bf16),
            pltpu.VMEM((M, HG, D), bf16),
            pltpu.VMEM((DC, HG, D), bf16),
            pltpu.VMEM((DC, HG, D), bf16),
            pltpu.VMEM((M * 8, D), u32),
            pltpu.VMEM((DC * 8, D), u32),
            pltpu.VMEM((DC * 8, D), u32),
            pltpu.VMEM((2, 3, S, D), bf16),
            pltpu.VMEM((BQ, CB * BQ + BQ // 2), f32),
            pltpu.VMEM((BQ // 2, BQ // 2), f32),
            pltpu.VMEM((BQ, 1), f32),
            pltpu.VMEM((S, M), bf16),
            pltpu.VMEM((H, S, D), bf16),
            pltpu.VMEM((H * D, M), bf16),
            pltpu.VMEM((M, F), bf16),
            pltpu.VMEM((M, F), bf16),
            pltpu.VMEM((F, M), bf16),
            pltpu.VMEM((S, M), bf16),
            pltpu.VMEM((S, M), bf16),
            pltpu.VMEM((S, 1), f32),
            pltpu.SemaphoreType.DMA((2,)),
            pltpu.SemaphoreType.DMA((3,)),
            pltpu.SemaphoreType.DMA((4,)),
            pltpu.SemaphoreType.DMA((S // RB,)),
        ],
        compiler_params=pltpu.CompilerParams(
            dimension_semantics=("arbitrary",), vmem_limit_bytes=126 * 1024 * 1024),
    )(x, c, A_w_q, A_w_uk, A_w_uv, wr, wo, B_w_gate, B_w_up, B_w_down)
    return out.reshape(1, S, M)
```

```python
import numpy as np
import jax
import jax.numpy as jnp
from jax import lax
import jax.experimental.pallas as pl
import jax.experimental.pallas.tpu as pltpu

S, M, H, D, DC, F = 2048, 1024, 32, 128, 512, 3584
BQ = 256
PB = 256
RB = 256
CB = 0
ORDER = "q7,p,e0,p,q6,p,e7,q5,e6,p,q4,p,e5,q2,p,e4,p,q3,q1,e2,p,e3,N,e1".split(",")
LOG2E = float(np.log2(np.e))
NT = (((1,), (1,)), ((), ()))
f32, bf16, u32 = jnp.float32, jnp.bfloat16, jnp.uint32
HG = 16


def _ln(v):
    m = jnp.mean(v, axis=-1, keepdims=True)
    d = v - m
    var = jnp.mean(d * d, axis=-1, keepdims=True)
    return d * lax.rsqrt(var + 1e-5)


def _dot(a, b):
    return jnp.dot(a, b, preferred_element_type=f32)


def _dot_cols(a, w_ref):
    return jnp.concatenate([_dot(a, w_ref[j]) for j in range(w_ref.shape[0])], axis=1)


def _dot_nt(a, b):
    return lax.dot_general(a, b, NT, preferred_element_type=f32)


def _kernel(x_hbm, c_hbm, wq_hbm, wk_hbm, wv_hbm, wr_ref, wo_hbm, wg_hbm, wu_hbm, wd_hbm,
            o_hbm,
            x_ref, c_ref, nq_ref, nk_ref, nv_ref, uq_ref, uk_ref, uv_ref, qkv_ref, sn_ref, sb_ref, mn_ref,
            xn_ref, ctx_ref, wo_ref, wg_ref, wu_ref, wd_ref, h_ref, st_ref, r_ref, a_ref,
            isem, nsem, wsem, osem):
    step = pl.program_id(0)

    def nat_copy(i, g):
        src, dst = ((wq_hbm, nq_ref), (wk_hbm, nk_ref), (wv_hbm, nv_ref))[i]
        return pltpu.make_async_copy(src.at[:, pl.ds(g * HG, HG), :], dst, nsem.at[i])

    NCH = S // PB

    def in_copy(i, j):
        src, dst = ((x_hbm, x_ref), (c_hbm, c_ref))[i]
        rows = pl.ds(j * PB, PB)
        return pltpu.make_async_copy(src.at[rows, :], dst.at[rows, :], isem.at[i, j])

    def w_copy(i):
        src, dst = ((wo_hbm, wo_ref), (wg_hbm, wg_ref), (wu_hbm, wu_ref), (wd_hbm, wd_ref))[i]
        if i == 0:
            return [pltpu.make_async_copy(src, dst, wsem.at[i])]
        return [pltpu.make_async_copy(src.at[:, pl.ds(j * 128, 128)], dst.at[j], wsem.at[i])
                for j in range(dst.shape[0])]

    def stage(j):
        nat, dst = ((nq_ref, uq_ref), (nk_ref, uk_ref), (nv_ref, uv_ref))[j]

        def body(i, carry):
            r = pl.multiple_of(i * 128, 128)
            v = pltpu.bitcast(nat[pl.ds(r, 128)], u32)
            n = 128 * HG // 2
            dst[pl.ds(pl.multiple_of(i * n, n), n), :] = v.reshape(n, 128)
            return carry
        lax.fori_loop(0, nat.shape[0] // 128, body, 0)

    def head_w(ref, hd):
        hl = hd % HG
        u = ref[pl.ds(hl // 2, ref.shape[0] * 2 // HG, stride=HG // 2), :]
        sh = jnp.asarray(16 * (1 - hl % 2)).astype(u32)
        return pltpu.bitcast((u << sh) & u32(0xFFFF0000), f32).astype(bf16)

    def proj_kv(hd):
        slot = hd % 2
        wk, wv = head_w(uk_ref, hd), head_w(uv_ref, hd)

        def chunk(i):
            rows = slice(i * PB, (i + 1) * PB)
            c = c_ref[rows, :]
            qkv_ref[slot, 1, rows, :] = _dot(c, wk).astype(bf16)
            qkv_ref[slot, 2, rows, :] = _dot(c, wv).astype(bf16)
        return chunk

    def proj_q(hd):
        slot = hd % 2
        wq = head_w(uq_ref, hd)

        def chunk(i):
            rows = slice(i * PB, (i + 1) * PB)
            qkv_ref[slot, 0, rows, :] = (_dot(xn_ref[rows, :], wq) * (D ** -0.5 * LOG2E)).astype(bf16)
        return chunk

    def proj(hd):
        kv, pq = proj_kv(hd), proj_q(hd)

        def chunk(i):
            kv(i)
            pq(i)
        return chunk

    HB = BQ // 2

    def scores(hd, i):
        slot = hd % 2
        r0, r1 = i * BQ, (i + 1) * BQ
        rm = r0 + HB
        q = qkv_ref[slot, 0, r0:r1, :]
        neg = -1e9 * LOG2E
        rr = lax.broadcasted_iota(jnp.int32, (BQ, HB), 0)
        cc = lax.broadcasted_iota(jnp.int32, (BQ, HB), 1)
        parts = []
        if r0 > 0:
            parts.append(_dot_nt(q, qkv_ref[slot, 1, 0:r0, :]))
        parts.append(jnp.where(cc <= rr, _dot_nt(q, qkv_ref[slot, 1, r0:rm, :]), neg))
        sa = jnp.concatenate(parts, axis=1) if len(parts) > 1 else parts[0]
        sb = jnp.where(cc[:HB] <= rr[:HB], _dot_nt(q[HB:], qkv_ref[slot, 1, rm:r1, :]), neg)
        ma = jnp.max(sa, axis=-1, keepdims=True)
        mb = jnp.maximum(ma[HB:], jnp.max(sb, axis=-1, keepdims=True))
        return sa, sb, jnp.concatenate([ma[:HB], mb], axis=0)

    def carry_scores(hd):
        sa, sb, m = scores(hd, CB)
        sn_ref[...] = sa
        sb_ref[...] = sb
        mn_ref[...] = m

    def softmax_pv(hd, i, sa, sb, m):
        slot = hd % 2
        r0, r1 = i * BQ, (i + 1) * BQ
        rm = r0 + HB
        pa = jnp.exp2(sa - m)
        pb = jnp.exp2(sb - m[HB:])
        la = jnp.sum(pa, axis=-1, keepdims=True)
        lb = la[HB:] + jnp.sum(pb, axis=-1, keepdims=True)
        oa = _dot(pa.astype(bf16), qkv_ref[slot, 2, 0:rm, :])
        ob = oa[HB:] + _dot(pb.astype(bf16), qkv_ref[slot, 2, rm:r1, :])
        ctx_ref[hd, r0:rm, :] = (oa[:HB] / la[:HB]).astype(bf16)
        ctx_ref[hd, rm:r1, :] = (ob / lb).astype(bf16)

    def attn_and_proj(hd, with_proj):
        chunk = proj(hd + 1) if with_proj else None
        done = 0
        pend = {}
        for tok in ORDER:
            if tok == "p":
                if with_proj:
                    chunk(done)
                done += 1
            elif tok == "N":
                if with_proj:
                    carry_scores(hd + 1)
            elif tok[0] == "q":
                pend[int(tok[1])] = scores(hd, int(tok[1]))
            else:
                i = int(tok[1])
                softmax_pv(hd, i, *(pend[i] if i in pend else (sn_ref[...], sb_ref[...], mn_ref[...])))
        assert done == S // PB

    @pl.when(step == 0)
    def _():
        for i in (1, 2, 0):
            nat_copy(i, 0).start()
        PRE = (0, 0, NCH, NCH)

        def start_in(a, b):
            for i in range(a, b):
                in_copy(1, i).start()
                in_copy(0, i).start()
        start_in(0, PRE[0])
        for n, i in enumerate((1, 2, 0)):
            nat_copy(i, 0).wait()
            start_in(PRE[n], PRE[n + 1])
            stage(i)
        chunk = proj(0)
        for i in range(NCH):
            in_copy(1, i).wait()
            in_copy(0, i).wait()
            rows = slice(i * PB, (i + 1) * PB)
            xn_ref[rows, :] = _ln(x_ref[rows, :].astype(f32)).astype(bf16)
            chunk(i)
        for i in range(3):
            nat_copy(i, 1).start()
        for i in range(4):
            [c.start() for c in w_copy(i)]
        carry_scores(0)

    @pl.when(step == HG - 1)
    def _():
        for i in range(3):
            nat_copy(i, 1).wait()
            stage(i)

    @pl.when(step < H - 1)
    def _():
        attn_and_proj(step, True)

    @pl.when(step == H - 1)
    def _():
        attn_and_proj(step, False)
        [c.wait() for c in w_copy(0)]
        wr = wr_ref[...].astype(f32)
        NQ = S // RB

        def ocopy(i):
            rows = pl.ds(pl.multiple_of(i * RB, RB) if not isinstance(i, int) else i * RB, RB)
            return pltpu.make_async_copy(st_ref.at[rows, :], o_hbm.at[rows, :], osem.at[i])

        lane = lax.broadcasted_iota(jnp.int32, (RB, 128), 1)
        rrow = lax.broadcasted_iota(jnp.int32, (RB, 128), 0)

        def oproj(i):
            rows = pl.ds(pl.multiple_of(i * RB, RB), RB)
            ctx = jnp.concatenate([ctx_ref[j, rows, :] for j in range(H)], axis=1)
            return _dot(ctx, wo_ref[...]).astype(bf16)

        def epilogue(i, a):
            rows = pl.ds(pl.multiple_of(i * RB, RB), RB)
            h = (x_ref[rows, :].astype(f32) + a.astype(f32)).astype(bf16)
            ln = _ln(h.astype(f32)).astype(bf16)
            r = jnp.sum(ln.astype(f32) * wr, axis=-1, keepdims=True).astype(bf16).astype(f32)
            r_ref[...] = jnp.where(lane == i, r, r_ref[...])
            h_ref[rows, :] = h
            xn_ref[rows, :] = ln
            st_ref[rows, :] = (h.astype(f32) + ln.astype(f32)).astype(bf16)

        r_ref[...] = jnp.full((RB, 128), -jnp.inf, f32)
        a_ref[...] = jnp.zeros((RB, M), bf16)

        def body(i, carry):
            a_prev = a_ref[...]
            a_ref[...] = oproj(i)
            epilogue(jnp.maximum(i - 1, 0), a_prev)

            @pl.when(i > 0)
            def _():
                ocopy(i - 1).start()
            return carry
        lax.fori_loop(0, NQ, body, 0)
        epilogue(NQ - 1, a_ref[...])
        ocopy(NQ - 1).start()

        r = r_ref[...]
        ids = lane * RB + rrow
        m1 = jnp.max(r)
        i1 = jnp.min(jnp.where(r == m1, ids, S))
        r2 = jnp.where(ids == i1, -jnp.inf, r)
        m2 = jnp.max(r2)
        i2 = jnp.min(jnp.where(r2 == m2, ids, S))
        i1 = jnp.minimum(i1, S - 1)
        i2 = jnp.minimum(i2, S - 1)
        b1 = pl.multiple_of((i1 // 16) * 16, 16)
        b2 = pl.multiple_of((i2 // 16) * 16, 16)
        rid = lax.broadcasted_iota(jnp.int32, (16, 1), 0)
        t1 = xn_ref[pl.ds(b1, 16), :].astype(f32)
        t2 = xn_ref[pl.ds(b2, 16), :].astype(f32)
        x1 = jnp.sum(jnp.where(rid == i1 - b1, t1, 0.0), axis=0, keepdims=True)
        x2 = jnp.sum(jnp.where(rid == i2 - b2, t2, 0.0), axis=0, keepdims=True)
        xs = jnp.where(rid == 0, x1, jnp.where(rid == 1, x2, 0.0)).astype(bf16)
        for i in range(1, 4):
            [c.wait() for c in w_copy(i)]
        g = _dot_cols(xs, wg_ref).astype(bf16).astype(f32)
        u = _dot_cols(xs, wu_ref).astype(bf16).astype(f32)
        g = (g * jax.nn.sigmoid(g)).astype(bf16).astype(f32)
        y = _dot_cols((g * u).astype(bf16), wd_ref).astype(bf16).astype(f32)
        s1 = jax.nn.sigmoid(jnp.full((1, M), m1, f32)).astype(bf16).astype(f32)
        s2 = jax.nn.sigmoid(jnp.full((1, M), m2, f32)).astype(bf16).astype(f32)
        y1 = (y[0:1] * s1).astype(bf16).astype(f32)
        y2 = (y[1:2] * s2).astype(bf16).astype(f32)
        for i in range(NQ):
            ocopy(i).wait()
        for (bb, ii, tt, yy) in ((b1, i1, t1, y1), (b2, i2, t2, y2)):
            rows = pl.ds(bb, 16)
            new = (h_ref[rows, :].astype(f32) + (tt + yy).astype(bf16).astype(f32)).astype(bf16)
            st_ref[rows, :] = jnp.where(rid == ii - bb, new, st_ref[rows, :])

        def patch(bb, k):
            rows = pl.ds(bb, 16)
            return pltpu.make_async_copy(st_ref.at[rows, :], o_hbm.at[rows, :], osem.at[k])

        patch(b2, 1).start()

        @pl.when(b1 != b2)
        def _():
            patch(b1, 0).start()
            patch(b1, 0).wait()
        patch(b2, 1).wait()


@jax.jit
def pallas_sequential_preLN__compressed_kv_cla__moe_arch_mod__prompt_kernel(
        A_x, A_c_kv, A_w_q, A_w_uk, A_w_uv, A_w_o, B_x, B_w_r, B_w_gate, B_w_up, B_w_down):
    x = A_x.reshape(S, M)
    c = A_c_kv.reshape(S, DC)
    wo = A_w_o.reshape(H * D, M)
    wr = B_w_r.reshape(1, M)
    anyspec = pl.BlockSpec(memory_space=pl.ANY)
    out = pl.pallas_call(
        _kernel,
        grid=(H,),
        in_specs=[anyspec] * 5 + [pl.BlockSpec((1, M), lambda h: (0, 0))] + [anyspec] * 4,
        out_specs=anyspec,
        out_shape=jax.ShapeDtypeStruct((S, M), bf16),
        scratch_shapes=[
            pltpu.VMEM((S, M), bf16),
            pltpu.VMEM((S, DC), bf16),
            pltpu.VMEM((M, HG, D), bf16),
            pltpu.VMEM((DC, HG, D), bf16),
            pltpu.VMEM((DC, HG, D), bf16),
            pltpu.VMEM((M * HG // 2, D), u32),
            pltpu.VMEM((DC * HG // 2, D), u32),
            pltpu.VMEM((DC * HG // 2, D), u32),
            pltpu.VMEM((2, 3, S, D), bf16),
            pltpu.VMEM((BQ, CB * BQ + BQ // 2), f32),
            pltpu.VMEM((BQ // 2, BQ // 2), f32),
            pltpu.VMEM((BQ, 1), f32),
            pltpu.VMEM((S, M), bf16),
            pltpu.VMEM((H, S, D), bf16),
            pltpu.VMEM((H * D, M), bf16),
            pltpu.VMEM((F // 128, M, 128), bf16),
            pltpu.VMEM((F // 128, M, 128), bf16),
            pltpu.VMEM((M // 128, F, 128), bf16),
            pltpu.VMEM((S, M), bf16),
            pltpu.VMEM((S, M), bf16),
            pltpu.VMEM((RB, 128), f32),
            pltpu.VMEM((RB, M), bf16),
            pltpu.SemaphoreType.DMA((2, S // PB)),
            pltpu.SemaphoreType.DMA((3,)),
            pltpu.SemaphoreType.DMA((4,)),
            pltpu.SemaphoreType.DMA((S // RB,)),
        ],
        compiler_params=pltpu.CompilerParams(
            dimension_semantics=("arbitrary",), vmem_limit_bytes=126 * 1024 * 1024),
    )(x, c, A_w_q, A_w_uk, A_w_uv, wr, wo, B_w_gate, B_w_up, B_w_down)
    return out.reshape(1, S, M)
```

```python
import numpy as np
import jax
import jax.numpy as jnp
from jax import lax
import jax.experimental.pallas as pl
import jax.experimental.pallas.tpu as pltpu

S, M, H, D, DC, F = 2048, 1024, 32, 128, 512, 3584
BQ = 256
PB = 256
RB = 256
CB = 0
ORDER = ("q7,k,v,u,e0,k,v,u,q6,k,v,u,e7,q5,"
         "e6,k,u,q4,e5,q2,v,k,v,u,k,u,v,e4,"
         "k,v,u,q3,q1,u,e2,k,v,e3,N,e1").split(",")
LOG2E = float(np.log2(np.e))
NT = (((1,), (1,)), ((), ()))
f32, bf16, u32 = jnp.float32, jnp.bfloat16, jnp.uint32
HG = 16


def _ln(v):
    m = jnp.mean(v, axis=-1, keepdims=True)
    d = v - m
    var = jnp.mean(d * d, axis=-1, keepdims=True)
    return d * lax.rsqrt(var + 1e-5)


def _dot(a, b):
    return jnp.dot(a, b, preferred_element_type=f32)


def _dot_cols(a, w_ref):
    return jnp.concatenate([_dot(a, w_ref[j]) for j in range(w_ref.shape[0])], axis=1)


def _dot_nt(a, b):
    return lax.dot_general(a, b, NT, preferred_element_type=f32)


def _kernel(x_hbm, c_hbm, wq_hbm, wk_hbm, wv_hbm, wr_ref, wo_hbm, wg_hbm, wu_hbm, wd_hbm,
            o_hbm,
            x_ref, c_ref, nq_ref, nk_ref, nv_ref, uq_ref, uk_ref, uv_ref, qkv_ref, sn_ref, sb_ref, mn_ref,
            xn_ref, ctx_ref, wo_ref, wg_ref, wu_ref, wd_ref, h_ref, st_ref, r_ref, a_ref,
            isem, nsem, wsem, osem):
    step = pl.program_id(0)

    def nat_copy(i, g):
        src, dst = ((wq_hbm, nq_ref), (wk_hbm, nk_ref), (wv_hbm, nv_ref))[i]
        return pltpu.make_async_copy(src.at[:, pl.ds(g * HG, HG), :], dst, nsem.at[i])

    NCH = S // PB

    def in_copy(i, j):
        src, dst = ((x_hbm, x_ref), (c_hbm, c_ref))[i]
        rows = pl.ds(j * PB, PB)
        return pltpu.make_async_copy(src.at[rows, :], dst.at[rows, :], isem.at[i, j])

    def w_copy(i):
        src, dst = ((wo_hbm, wo_ref), (wg_hbm, wg_ref), (wu_hbm, wu_ref), (wd_hbm, wd_ref))[i]
        if i == 0:
            return [pltpu.make_async_copy(src, dst, wsem.at[i])]
        return [pltpu.make_async_copy(src.at[:, pl.ds(j * 128, 128)], dst.at[j], wsem.at[i])
                for j in range(dst.shape[0])]

    def stage(j):
        nat, dst = ((nq_ref, uq_ref), (nk_ref, uk_ref), (nv_ref, uv_ref))[j]

        def body(i, carry):
            r = pl.multiple_of(i * 128, 128)
            v = pltpu.bitcast(nat[pl.ds(r, 128)], u32)
            n = 128 * HG // 2
            dst[pl.ds(pl.multiple_of(i * n, n), n), :] = v.reshape(n, 128)
            return carry
        lax.fori_loop(0, nat.shape[0] // 128, body, 0)

    def head_w(ref, hd):
        hl = hd % HG
        u = ref[pl.ds(hl // 2, ref.shape[0] * 2 // HG, stride=HG // 2), :]
        sh = jnp.asarray(16 * (1 - hl % 2)).astype(u32)
        return pltpu.bitcast((u << sh) & u32(0xFFFF0000), f32).astype(bf16)

    def proj(hd):
        slot = hd % 2

        def mk(idx, src, w, scale):
            def f(i):
                rows = slice(i * PB, (i + 1) * PB)
                y = _dot(src[rows, :], w)
                qkv_ref[slot, idx, rows, :] = (y * scale if scale else y).astype(bf16)
            return f
        return (mk(1, c_ref, head_w(uk_ref, hd), None), mk(2, c_ref, head_w(uv_ref, hd), None),
                mk(0, xn_ref, head_w(uq_ref, hd), D ** -0.5 * LOG2E))

    HB = BQ // 2

    def scores(hd, i):
        slot = hd % 2
        r0, r1 = i * BQ, (i + 1) * BQ
        rm = r0 + HB
        q = qkv_ref[slot, 0, r0:r1, :]
        neg = -1e9 * LOG2E
        rr = lax.broadcasted_iota(jnp.int32, (BQ, HB), 0)
        cc = lax.broadcasted_iota(jnp.int32, (BQ, HB), 1)
        parts = []
        if r0 > 0:
            parts.append(_dot_nt(q, qkv_ref[slot, 1, 0:r0, :]))
        parts.append(jnp.where(cc <= rr, _dot_nt(q, qkv_ref[slot, 1, r0:rm, :]), neg))
        sa = jnp.concatenate(parts, axis=1) if len(parts) > 1 else parts[0]
        sb = jnp.where(cc[:HB] <= rr[:HB], _dot_nt(q[HB:], qkv_ref[slot, 1, rm:r1, :]), neg)
        ma = jnp.max(sa, axis=-1, keepdims=True)
        mb = jnp.maximum(ma[HB:], jnp.max(sb, axis=-1, keepdims=True))
        return sa, sb, jnp.concatenate([ma[:HB], mb], axis=0)

    def carry_scores(hd):
        sa, sb, m = scores(hd, CB)
        sn_ref[...] = sa
        sb_ref[...] = sb
        mn_ref[...] = m

    def softmax_pv(hd, i, sa, sb, m):
        slot = hd % 2
        r0, r1 = i * BQ, (i + 1) * BQ
        rm = r0 + HB
        pa = jnp.exp2(sa - m)
        pb = jnp.exp2(sb - m[HB:])
        la = jnp.sum(pa, axis=-1, keepdims=True)
        lb = la[HB:] + jnp.sum(pb, axis=-1, keepdims=True)
        oa = _dot(pa.astype(bf16), qkv_ref[slot, 2, 0:rm, :])
        ob = oa[HB:] + _dot(pb.astype(bf16), qkv_ref[slot, 2, rm:r1, :])
        ctx_ref[hd, r0:rm, :] = (oa[:HB] / la[:HB]).astype(bf16)
        ctx_ref[hd, rm:r1, :] = (ob / lb).astype(bf16)

    def attn_and_proj(hd, with_proj):
        sub = dict(zip("kvu", proj(hd + 1))) if with_proj else None
        cnt = {"k": 0, "v": 0, "u": 0}
        pend = {}
        for tok in ORDER:
            if tok in cnt:
                if with_proj:
                    sub[tok](cnt[tok])
                cnt[tok] += 1
            elif tok == "N":
                if with_proj:
                    carry_scores(hd + 1)
            elif tok[0] == "q":
                pend[int(tok[1])] = scores(hd, int(tok[1]))
            else:
                i = int(tok[1])
                softmax_pv(hd, i, *(pend[i] if i in pend else (sn_ref[...], sb_ref[...], mn_ref[...])))
        assert all(n == S // PB for n in cnt.values())

    @pl.when(step == 0)
    def _():
        for i in (1, 2, 0):
            nat_copy(i, 0).start()
        PRE = (0, 0, NCH, NCH)

        def start_in(a, b):
            for i in range(a, b):
                in_copy(1, i).start()
                in_copy(0, i).start()
        start_in(0, PRE[0])
        for n, i in enumerate((1, 2, 0)):
            nat_copy(i, 0).wait()
            start_in(PRE[n], PRE[n + 1])
            stage(i)
        first = proj(0)
        for i in range(NCH):
            in_copy(1, i).wait()
            in_copy(0, i).wait()
            rows = slice(i * PB, (i + 1) * PB)
            xn_ref[rows, :] = _ln(x_ref[rows, :].astype(f32)).astype(bf16)
            for f in first:
                f(i)
        for i in range(3):
            nat_copy(i, 1).start()
        for i in range(4):
            [c.start() for c in w_copy(i)]
        carry_scores(0)

    @pl.when(step == HG - 1)
    def _():
        for i in range(3):
            nat_copy(i, 1).wait()
            stage(i)

    @pl.when(step < H - 1)
    def _():
        attn_and_proj(step, True)

    @pl.when(step == H - 1)
    def _():
        attn_and_proj(step, False)
        [c.wait() for c in w_copy(0)]
        wr = wr_ref[...].astype(f32)
        NQ = S // RB

        def ocopy(i):
            rows = pl.ds(pl.multiple_of(i * RB, RB) if not isinstance(i, int) else i * RB, RB)
            return pltpu.make_async_copy(st_ref.at[rows, :], o_hbm.at[rows, :], osem.at[i])

        lane = lax.broadcasted_iota(jnp.int32, (RB, 128), 1)
        rrow = lax.broadcasted_iota(jnp.int32, (RB, 128), 0)

        def oproj(i):
            rows = pl.ds(pl.multiple_of(i * RB, RB), RB)
            ctx = jnp.concatenate([ctx_ref[j, rows, :] for j in range(H)], axis=1)
            return _dot(ctx, wo_ref[...]).astype(bf16)

        def epilogue(i, a):
            rows = pl.ds(pl.multiple_of(i * RB, RB), RB)
            h = (x_ref[rows, :].astype(f32) + a.astype(f32)).astype(bf16)
            ln = _ln(h.astype(f32)).astype(bf16)
            r = jnp.sum(ln.astype(f32) * wr, axis=-1, keepdims=True).astype(bf16).astype(f32)
            r_ref[...] = jnp.where(lane == i, r, r_ref[...])
            h_ref[rows, :] = h
            xn_ref[rows, :] = ln
            st_ref[rows, :] = (h.astype(f32) + ln.astype(f32)).astype(bf16)

        r_ref[...] = jnp.full((RB, 128), -jnp.inf, f32)
        a_ref[...] = jnp.zeros((RB, M), bf16)

        def body(i, carry):
            a_prev = a_ref[...]
            a_ref[...] = oproj(i)
            epilogue(jnp.maximum(i - 1, 0), a_prev)

            @pl.when(i > 0)
            def _():
                ocopy(i - 1).start()
            return carry
        lax.fori_loop(0, NQ, body, 0)
        epilogue(NQ - 1, a_ref[...])
        ocopy(NQ - 1).start()

        r = r_ref[...]
        ids = lane * RB + rrow
        m1 = jnp.max(r)
        i1 = jnp.min(jnp.where(r == m1, ids, S))
        r2 = jnp.where(ids == i1, -jnp.inf, r)
        m2 = jnp.max(r2)
        i2 = jnp.min(jnp.where(r2 == m2, ids, S))
        i1 = jnp.minimum(i1, S - 1)
        i2 = jnp.minimum(i2, S - 1)
        b1 = pl.multiple_of((i1 // 16) * 16, 16)
        b2 = pl.multiple_of((i2 // 16) * 16, 16)
        rid = lax.broadcasted_iota(jnp.int32, (16, 1), 0)
        t1 = xn_ref[pl.ds(b1, 16), :].astype(f32)
        t2 = xn_ref[pl.ds(b2, 16), :].astype(f32)
        x1 = jnp.sum(jnp.where(rid == i1 - b1, t1, 0.0), axis=0, keepdims=True)
        x2 = jnp.sum(jnp.where(rid == i2 - b2, t2, 0.0), axis=0, keepdims=True)
        xs = jnp.where(rid == 0, x1, jnp.where(rid == 1, x2, 0.0)).astype(bf16)
        for i in range(1, 4):
            [c.wait() for c in w_copy(i)]
        g = _dot_cols(xs, wg_ref).astype(bf16).astype(f32)
        u = _dot_cols(xs, wu_ref).astype(bf16).astype(f32)
        g = (g * jax.nn.sigmoid(g)).astype(bf16).astype(f32)
        y = _dot_cols((g * u).astype(bf16), wd_ref).astype(bf16).astype(f32)
        s1 = jax.nn.sigmoid(jnp.full((1, M), m1, f32)).astype(bf16).astype(f32)
        s2 = jax.nn.sigmoid(jnp.full((1, M), m2, f32)).astype(bf16).astype(f32)
        y1 = (y[0:1] * s1).astype(bf16).astype(f32)
        y2 = (y[1:2] * s2).astype(bf16).astype(f32)
        for i in range(NQ):
            ocopy(i).wait()
        for (bb, ii, tt, yy) in ((b1, i1, t1, y1), (b2, i2, t2, y2)):
            rows = pl.ds(bb, 16)
            new = (h_ref[rows, :].astype(f32) + (tt + yy).astype(bf16).astype(f32)).astype(bf16)
            st_ref[rows, :] = jnp.where(rid == ii - bb, new, st_ref[rows, :])

        def patch(bb, k):
            rows = pl.ds(bb, 16)
            return pltpu.make_async_copy(st_ref.at[rows, :], o_hbm.at[rows, :], osem.at[k])

        patch(b2, 1).start()

        @pl.when(b1 != b2)
        def _():
            patch(b1, 0).start()
            patch(b1, 0).wait()
        patch(b2, 1).wait()


@jax.jit
def pallas_sequential_preLN__compressed_kv_cla__moe_arch_mod__prompt_kernel(
        A_x, A_c_kv, A_w_q, A_w_uk, A_w_uv, A_w_o, B_x, B_w_r, B_w_gate, B_w_up, B_w_down):
    x = A_x.reshape(S, M)
    c = A_c_kv.reshape(S, DC)
    wo = A_w_o.reshape(H * D, M)
    wr = B_w_r.reshape(1, M)
    anyspec = pl.BlockSpec(memory_space=pl.ANY)
    out = pl.pallas_call(
        _kernel,
        grid=(H,),
        in_specs=[anyspec] * 5 + [pl.BlockSpec((1, M), lambda h: (0, 0))] + [anyspec] * 4,
        out_specs=anyspec,
        out_shape=jax.ShapeDtypeStruct((S, M), bf16),
        scratch_shapes=[
            pltpu.VMEM((S, M), bf16),
            pltpu.VMEM((S, DC), bf16),
            pltpu.VMEM((M, HG, D), bf16),
            pltpu.VMEM((DC, HG, D), bf16),
            pltpu.VMEM((DC, HG, D), bf16),
            pltpu.VMEM((M * HG // 2, D), u32),
            pltpu.VMEM((DC * HG // 2, D), u32),
            pltpu.VMEM((DC * HG // 2, D), u32),
            pltpu.VMEM((2, 3, S, D), bf16),
            pltpu.VMEM((BQ, CB * BQ + BQ // 2), f32),
            pltpu.VMEM((BQ // 2, BQ // 2), f32),
            pltpu.VMEM((BQ, 1), f32),
            pltpu.VMEM((S, M), bf16),
            pltpu.VMEM((H, S, D), bf16),
            pltpu.VMEM((H * D, M), bf16),
            pltpu.VMEM((F // 128, M, 128), bf16),
            pltpu.VMEM((F // 128, M, 128), bf16),
            pltpu.VMEM((M // 128, F, 128), bf16),
            pltpu.VMEM((S, M), bf16),
            pltpu.VMEM((S, M), bf16),
            pltpu.VMEM((RB, 128), f32),
            pltpu.VMEM((RB, M), bf16),
            pltpu.SemaphoreType.DMA((2, S // PB)),
            pltpu.SemaphoreType.DMA((3,)),
            pltpu.SemaphoreType.DMA((4,)),
            pltpu.SemaphoreType.DMA((S // RB,)),
        ],
        compiler_params=pltpu.CompilerParams(
            dimension_semantics=("arbitrary",), vmem_limit_bytes=126 * 1024 * 1024),
    )(x, c, A_w_q, A_w_uk, A_w_uv, wr, wo, B_w_gate, B_w_up, B_w_down)
    return out.reshape(1, S, M)
```
